```python
import os as _os
_os.environ.setdefault("JAX_PLATFORMS", "cpu")
import jax
import jax.numpy as jnp

def _softmax(x, axis=-1):
    return jax.nn.softmax(x, axis=axis)
def _gelu(x):
    return jax.nn.gelu(x, approximate=True)
def _silu(x):
    return jax.nn.silu(x)
def _sigmoid(x):
    return jax.nn.sigmoid(x)
def _layernorm(x, axis=-1, eps=1e-5):
    m = jnp.mean(x, axis=axis, keepdims=True)
    v = jnp.var(x, axis=axis, keepdims=True)
    return (x - m) / jnp.sqrt(v + eps)
def _scatter_add(tgt, idx, src, axis=0):
    return tgt.at[idx].add(src)
def _segment_sum(src, seg, n):
    return jax.ops.segment_sum(src, seg, n)
class _Rng:
    def __init__(self, key):
        self._k = key
    def _next(self):
        self._k, sub = jax.random.split(self._k)
        return sub
    def normal(self, shape):
        return jax.random.normal(self._next(), shape, dtype=jnp.bfloat16)
    def randint(self, lo, hi, shape):
        return jax.random.randint(self._next(), shape, lo, hi, dtype=jnp.int32)
    def uniform(self, shape, lo=0.0, hi=1.0):
        return jax.random.uniform(self._next(), shape, jnp.bfloat16, lo, hi)
    def permutation(self, n):
        return jax.random.permutation(self._next(), n)


kernel_name = 'standalone__gqa_softmax__near_ridge'

def setup_inputs():
    _rng = _Rng(jax.random.key(int.from_bytes(__import__("os").urandom(4), "little")))
    _w = (lambda a: (lambda t: t.astype(jnp.bfloat16) if jnp.issubdtype(t.dtype, jnp.floating) else t)(jnp.asarray(a)))
    B, Hq, Hkv, Sq, Sk, D = 8, 16, 8, 512, 512, 256
    return {
        "q": _w((lambda *s: _rng.normal(s) * 0.4)(B, Hq, Sq, D)),
        "k": _w((lambda *s: _rng.normal(s) * 0.4)(B, Hkv, Sk, D)),
        "v": _w((lambda *s: _rng.normal(s) * 0.05)(B, Hkv, Sk, D)),
    }

def reference(q, k, v):
    B, Hq, Sq, D = q.shape
    Hkv = k.shape[1]
    rep = Hq // Hkv
    k = jnp.repeat(k, rep, axis=1)
    v = jnp.repeat(v, rep, axis=1)
    scale = D ** -0.5
    scores = jnp.einsum("bhqd,bhkd->bhqk", q, k) * scale
    p = _softmax(scores, axis=-1)
    return jnp.einsum("bhqk,bhkd->bhqd", p, v)
```

```python
import functools

import jax
import jax.numpy as jnp
import jax.experimental.pallas as pl
import jax.experimental.pallas.tpu as pltpu


def _attn_kernel(q_ref, k_ref, v_ref, o_ref, *, scale):
    q = q_ref[0]
    k = k_ref[0]
    v = v_ref[0]
    s = jax.lax.dot_general(
        q, k, (((1,), (1,)), ((), ())), preferred_element_type=jnp.float32
    )
    m = jnp.max(s, axis=-1, keepdims=True)
    p = jnp.exp((s - m) * scale)
    l = jnp.sum(p, axis=-1, keepdims=True)
    o = jnp.dot(p.astype(jnp.bfloat16), v, preferred_element_type=jnp.float32)
    o_ref[0] = (o / l).astype(o_ref.dtype)


@jax.jit
def pallas_standalone__gqa_softmax__near_ridge_kernel(
    q: jax.Array,
    k: jax.Array,
    v: jax.Array,
):
    B, Hq, Sq, D = q.shape
    _, Hkv, Sk, _ = k.shape
    rep = Hq // Hkv
    G = B * Hkv
    qg = q.reshape(G, rep * Sq, D)
    kg = k.reshape(G, Sk, D)
    vg = v.reshape(G, Sk, D)
    scale = float(D) ** -0.5

    out = pl.pallas_call(
        functools.partial(_attn_kernel, scale=scale),
        grid=(G,),
        in_specs=[
            pl.BlockSpec((1, rep * Sq, D), lambda g: (g, 0, 0)),
            pl.BlockSpec((1, Sk, D), lambda g: (g, 0, 0)),
            pl.BlockSpec((1, Sk, D), lambda g: (g, 0, 0)),
        ],
        out_specs=pl.BlockSpec((1, rep * Sq, D), lambda g: (g, 0, 0)),
        out_shape=jax.ShapeDtypeStruct((G, rep * Sq, D), q.dtype),
        compiler_params=pltpu.CompilerParams(
            dimension_semantics=("parallel",),
            vmem_limit_bytes=64 * 1024 * 1024,
        ),
    )(qg, kg, vg)
    return out.reshape(B, Hq, Sq, D)
```

```python
import functools, math
import jax
import jax.numpy as jnp
from jax import lax
import jax.experimental.pallas as pl
import jax.experimental.pallas.tpu as pltpu


def make_ramp(kind):
    if kind == 'A':
        return [
            ([('k', 0, 1), ('qh', 0, 0)], [('qk', 0, 0, 512)]),
            ([('qh', 0, 1), ('v', 0, 1)], [('qk', 0, 512, 512), ('pv', 0, 0, 512), ('pv', 0, 512, 512)]),
            ([('k', 1, 1), ('q', 1, 1), ('v', 1, 1), ('k', 2, 1), ('qh', 2, 0)],
             [('qk', 1, 0, 1024), ('qk', 2, 0, 512), ('pv', 1, 0, 1024)]),
            ([('qh', 2, 1), ('v', 2, 1), ('k', 3, 2), ('q', 3, 2), ('v', 3, 2)],
             [('pv', 2, 0, 512), ('qk', 2, 512, 512), ('qk', 3, 0, 1024), ('pv', 2, 512, 512), ('qk', 4, 0, 1024),
              ('pv', 3, 0, 1024), ('pv', 4, 0, 1024)]),
            ([('k', 5, 3), ('q', 5, 3), ('v', 5, 3)],
             [('qk', 5, 0, 1024), ('qk', 6, 0, 1024), ('pv', 5, 0, 1024), ('qk', 7, 0, 1024),
              ('pv', 6, 0, 1024), ('pv', 7, 0, 1024)]),
        ], 8
    if kind == 'B':
        return [
            ([('k', 0, 1), ('q', 0, 1), ('v', 0, 1)], [('qk', 0, 0, 512), ('qk', 0, 512, 512), ('pv', 0, 0, 512), ('pv', 0, 512, 512)]),
            ([('k', 1, 2), ('q', 1, 2), ('v', 1, 2)], [('qk', 1, 0, 1024), ('qk', 2, 0, 1024), ('pv', 1, 0, 1024), ('pv', 2, 0, 1024)]),
            ([('k', 3, 5), ('q', 3, 5), ('v', 3, 5)],
             [('qk', 3, 0, 1024), ('qk', 4, 0, 1024), ('pv', 3, 0, 1024), ('qk', 5, 0, 1024), ('pv', 4, 0, 1024),
              ('qk', 6, 0, 1024), ('pv', 5, 0, 1024), ('qk', 7, 0, 1024), ('pv', 6, 0, 1024), ('pv', 7, 0, 1024)]),
        ], 8


def _attn_kernel(q_hbm, k_hbm, v_hbm, o_hbm, buf, isem, osem,
                 *, c, kind, gs, G, oc, defer, upfront):
    ramp, R = make_ramp(kind)
    nsteady = (G - R) // gs
    nr = len(ramp)
    RQ, SK = 1024, 512
    K0, V0 = RQ, RQ + SK

    def piece_copy(p, sem):
        if p[0] == 'k':
            return pltpu.make_async_copy(k_hbm.at[pl.ds(p[1], p[2])], buf.at[pl.ds(p[1], p[2]), pl.ds(K0, SK)], sem)
        if p[0] == 'v':
            return pltpu.make_async_copy(v_hbm.at[pl.ds(p[1], p[2])], buf.at[pl.ds(p[1], p[2]), pl.ds(V0, SK)], sem)
        if p[0] == 'q':
            return pltpu.make_async_copy(q_hbm.at[pl.ds(p[1], p[2])], buf.at[pl.ds(p[1], p[2]), pl.ds(0, RQ)], sem)
        if p[0] == 'qh':
            return pltpu.make_async_copy(q_hbm.at[p[1], pl.ds(p[2] * 512, 512)], buf.at[p[1], pl.ds(p[2] * 512, 512)], sem)

    def steady_start(s):
        a = R + s * gs
        for kind_ in 'kqv':
            piece_copy((kind_, a, gs), isem.at[nr + s]).start()

    def qk(j, r0, t):
        return lax.dot_general(buf[j, r0:r0 + t, :], buf[j, K0:K0 + SK, :], (((1,), (1,)), ((), ())),
                               preferred_element_type=jnp.float32)

    def softmax(s):
        m = jnp.max(s, axis=-1, keepdims=True)
        p = jnp.exp2((s - m) * c)
        l = jnp.sum(p, axis=-1, keepdims=True)
        r = pl.reciprocal(l, approx=True)
        r = r * (2.0 - l * r)
        return (p * r).astype(jnp.bfloat16)

    def pv(p, j, r0, t, send):
        o = jnp.dot(p, buf[j, V0:V0 + SK, :], preferred_element_type=jnp.float32).astype(buf.dtype)
        occ = min(oc, t)
        for u in range(t // occ):
            a = r0 + u * occ
            buf[j, a:a + occ, :] = o[u * occ:(u + 1) * occ]
            if send:
                pltpu.make_async_copy(buf.at[j, pl.ds(a, occ)], o_hbm.at[j, pl.ds(a, occ)], osem.at[0]).start()

    def run_ops(ops, svals, base, send):
        pending = [key for key in svals if svals[key][0] == 's']
        for n, op in enumerate(ops):
            name, j, r0, t = op
            if name == 'qk':
                svals[(j, r0)] = ('s', qk(base + j, r0, t))
            else:
                tag, val = svals.pop((j, r0))
                if tag == 's':
                    val = softmax(val)
                pv(val, base + j, r0, t, send)
            if n + 1 < len(ops):
                for key in list(svals):
                    if svals[key][0] == 's':
                        svals[key] = ('p', softmax(svals[key][1]))

    for b in range(nr):
        for p in ramp[b][0]:
            piece_copy(p, isem.at[b]).start()
    nup = nsteady if upfront else min(2, nsteady)
    for s in range(nup):
        steady_start(s)

    svals = {}
    for b in range(nr):
        for p in ramp[b][0]:
            piece_copy(p, isem.at[b]).wait()
        run_ops(ramp[b][1], svals, 0, not defer)
    assert not svals

    ops = [('qk', 0, 0, RQ)]
    for jj in range(gs):
        if jj + 1 < gs:
            ops.append(('qk', jj + 1, 0, RQ))
        ops.append(('pv', jj, 0, RQ))

    def body(s, carry):
        a = R + s * gs
        blk = buf.at[pl.ds(a, gs)]
        pltpu.make_async_copy(blk, blk, isem.at[nr + s]).wait()
        sv = {}
        run_ops(ops[:1], sv, a, True)
        if not upfront:
            @pl.when(s + 2 < nsteady)
            def _():
                steady_start(s + 2)
        if defer:
            nd = R // defer
            @pl.when(s < nd)
            def _():
                pltpu.make_async_copy(buf.at[pl.ds(s * defer, defer), pl.ds(0, RQ)],
                                      o_hbm.at[pl.ds(s * defer, defer)], osem.at[0]).start()
        run_ops(ops[1:], sv, a, True)
        return carry

    lax.fori_loop(0, nsteady, body, 0)
    pltpu.make_async_copy(buf.at[:, pl.ds(0, RQ)], o_hbm, osem.at[0]).wait()


def _build(kind='A', gs=8, nobc=True, oc=256, defer=2, upfront=True, nosem=True):
    def fn(q, k, v):
        B, Hq, Sq, D = q.shape
        _, Hkv, Sk, _ = k.shape
        rep = Hq // Hkv
        G = B * Hkv
        qg = q.reshape(G, rep * Sq, D)
        kg = k.reshape(G, Sk, D)
        vg = v.reshape(G, Sk, D)
        c = float(D) ** -0.5 * math.log2(math.e)
        ramp, R = make_ramp(kind)
        out = pl.pallas_call(
            functools.partial(_attn_kernel, c=c, kind=kind, gs=gs, G=G, oc=oc, defer=defer, upfront=upfront),
            in_specs=[pl.BlockSpec(memory_space=pl.ANY)] * 3,
            out_specs=pl.BlockSpec(memory_space=pl.ANY),
            out_shape=jax.ShapeDtypeStruct((G, rep * Sq, D), q.dtype),
            scratch_shapes=[
                pltpu.VMEM((G, rep * Sq + 2 * Sk, D), q.dtype),
                pltpu.SemaphoreType.DMA((len(ramp) + (G - R) // gs,)),
                pltpu.SemaphoreType.DMA((1,)),
            ],
            compiler_params=pltpu.CompilerParams(
                vmem_limit_bytes=120 * 1024 * 1024,
                disable_bounds_checks=nobc,
                disable_semaphore_checks=nosem,
            ),
        )(qg, kg, vg)
        return out.reshape(B, Hq, Sq, D)
    return fn


@jax.jit
def pallas_standalone__gqa_softmax__near_ridge_kernel(q: jax.Array, k: jax.Array, v: jax.Array):
    return _build()(q, k, v)
```

```python
import functools
import math

import jax
import jax.numpy as jnp
from jax import lax
import jax.experimental.pallas as pl
import jax.experimental.pallas.tpu as pltpu

_F = 1024
_H = _F // 2
_Q = _F // 4
_GS = 8
_R = 8
_DEFER = 2
_LAST_CHUNK = 128


def _qa(j, r=0, t=_F): return ("qka", j, r, t)
def _qb(j, r=0, t=_F): return ("qkb", j, r, t)
def _sm(j, r=0, t=_F): return ("sm", j, r, t)
def _pa(j, r=0, t=_F): return ("pva", j, r, t)
def _pb(j, r=0, t=_F): return ("pvb", j, r, t)
def _qk(j, r=0, t=_F): return ("qk", j, r, t)
def _pv(j, r=0, t=_F): return ("pv", j, r, t)


def _interleaved(js):
    ops = []
    for n, j in enumerate(js):
        ops.append(_qa(j))
        if n:
            ops.append(_pa(js[n - 1]))
        ops += [_qb(j), _sm(j)]
        if n:
            ops.append(_pb(js[n - 1]))
    return ops + [_pa(js[-1]), _pb(js[-1])]


_RAMP = (
    ([("k", 0, 1), ("qr", 0, 0, _H)],
     [_qk(0, 0, _Q), _sm(0, 0, _Q), _qk(0, _Q, _Q)]),
    ([("qr", 0, _H, _H), ("v", 0, 1)],
     [_pv(0, 0, _Q), _sm(0, _Q, _Q), _qk(0, _H, _H), _sm(0, _H, _H),
      _pv(0, _Q, _Q), _pv(0, _H, _H)]),
    ([("k", 1, 1), ("q", 1, 1), ("v", 1, 1), ("k", 2, 1), ("qr", 2, 0, _H)],
     [_qa(1), _qb(1), _sm(1), _qk(2, 0, _H), _pa(1)]),
    ([("qr", 2, _H, _H), ("v", 2, 1), ("k", 3, 1), ("q", 3, 1), ("v", 3, 1)],
     [_pb(1), _sm(2, 0, _H), _qk(2, _H, _H), _sm(2, _H, _H), _qa(3),
      _pv(2, 0, _H), _qb(3), _sm(3), _pv(2, _H, _H), _pa(3)]),
    ([("k", 4, 4), ("q", 4, 4), ("v", 4, 4)],
     [_pb(3)] + _interleaved([4, 5, 6, 7])),
)


def _attn_kernel(q_hbm, k_hbm, v_hbm, o_hbm, buf, isem, osem, *, c, sk, groups):
    d = buf.shape[2]
    k0, v0 = _F, _F + sk
    nsteady = (groups - _R) // _GS
    nr = len(_RAMP)
    nt = (((1,), (1,)), ((), ()))

    def piece_copy(p, sem):
        if p[0] == "qr":
            rows = pl.ds(p[2], p[3])
            return pltpu.make_async_copy(q_hbm.at[p[1], rows], buf.at[p[1], rows], sem)
        src, off, n = {"q": (q_hbm, 0, _F), "k": (k_hbm, k0, sk), "v": (v_hbm, v0, sk)}[p[0]]
        grp = pl.ds(p[1], p[2])
        return pltpu.make_async_copy(src.at[grp], buf.at[grp, pl.ds(off, n)], sem)

    def scores(j, r0, t, lo, hi):
        return lax.dot_general(buf[j, r0:r0 + t, :], buf[j, k0 + lo:k0 + hi, :], nt,
                               preferred_element_type=jnp.float32)

    def softmax(s):
        m = jnp.max(s, axis=-1, keepdims=True)
        p = jnp.exp2((s - m) * c)
        l = jnp.sum(p, axis=-1, keepdims=True)
        r = pl.reciprocal(l, approx=True)
        r = r * (2.0 - l * r)
        return (p * r).astype(jnp.bfloat16)

    def values(p, j, lo, hi):
        return jnp.dot(p, buf[j, v0:v0 + sk, lo:hi], preferred_element_type=jnp.float32)

    def store(o, j, r0, t, chunk):
        o = o.astype(buf.dtype)
        if not chunk:
            buf[j, r0:r0 + t, :] = o
            return
        for u in range(0, t, chunk):
            buf[j, r0 + u:r0 + u + chunk, :] = o[u:u + chunk]
            rows = pl.ds(r0 + u, chunk)
            pltpu.make_async_copy(buf.at[j, rows], o_hbm.at[j, rows], osem.at[0]).start()

    def run_ops(ops, vals, base, send, last=None):
        for op in ops:
            name, j, r0, t = op
            g, key = base + j, (j, r0)
            chunk = (_LAST_CHUNK if op == last else t) if send else 0
            if name == "qk":
                vals[key] = scores(g, r0, t, 0, sk)
            elif name == "qka":
                vals[key] = scores(g, r0, t, 0, sk // 2)
            elif name == "qkb":
                vals[key] = jnp.concatenate(
                    [vals[key], scores(g, r0, t, sk // 2, sk)], axis=1)
            elif name == "sm":
                vals[key] = softmax(vals[key])
            elif name == "pv":
                store(values(vals.pop(key), g, 0, d), g, r0, t, chunk)
            elif name == "pva":
                vals[key + ("o",)] = values(vals[key], g, 0, d // 2)
            else:
                o = jnp.concatenate(
                    [vals.pop(key + ("o",)), values(vals.pop(key), g, d // 2, d)], axis=1)
                store(o, g, r0, t, chunk)

    for b in range(nr):
        for p in _RAMP[b][0]:
            piece_copy(p, isem.at[b]).start()
    for s in range(nsteady):
        for name in "kqv":
            piece_copy((name, _R + s * _GS, _GS), isem.at[nr + s]).start()

    vals = {}
    for b in range(nr):
        for p in _RAMP[b][0]:
            piece_copy(p, isem.at[b]).wait()
        run_ops(_RAMP[b][1], vals, 0, False)
    assert not vals

    ops = _interleaved(list(range(_GS)))

    def body(s, carry):
        a = _R + s * _GS
        blk = buf.at[pl.ds(a, _GS)]
        pltpu.make_async_copy(blk, blk, isem.at[nr + s]).wait()
        sv = {}
        run_ops(ops[:1], sv, a, True)

        @pl.when(s < _R // _DEFER)
        def _():
            grp = pl.ds(s * _DEFER, _DEFER)
            pltpu.make_async_copy(buf.at[grp, pl.ds(0, _F)], o_hbm.at[grp], osem.at[0]).start()

        run_ops(ops[1:], sv, a, True, last=ops[-1])
        return carry

    lax.fori_loop(0, nsteady, body, 0)
    pltpu.make_async_copy(buf.at[:, pl.ds(0, _F)], o_hbm, osem.at[0]).wait()


@jax.jit
def pallas_standalone__gqa_softmax__near_ridge_kernel(
    q: jax.Array,
    k: jax.Array,
    v: jax.Array,
):
    B, Hq, Sq, D = q.shape
    _, Hkv, Sk, _ = k.shape
    rep = Hq // Hkv
    G = B * Hkv
    assert rep * Sq == _F and (G - _R) % _GS == 0 and (G - _R) // _GS >= _R // _DEFER
    c = float(D) ** -0.5 * math.log2(math.e)

    out = pl.pallas_call(
        functools.partial(_attn_kernel, c=c, sk=Sk, groups=G),
        in_specs=[pl.BlockSpec(memory_space=pl.ANY)] * 3,
        out_specs=pl.BlockSpec(memory_space=pl.ANY),
        out_shape=jax.ShapeDtypeStruct((G, _F, D), q.dtype),
        scratch_shapes=[
            pltpu.VMEM((G, _F + 2 * Sk, D), q.dtype),
            pltpu.SemaphoreType.DMA((len(_RAMP) + (G - _R) // _GS,)),
            pltpu.SemaphoreType.DMA((1,)),
        ],
        compiler_params=pltpu.CompilerParams(
            vmem_limit_bytes=120 * 1024 * 1024,
            disable_bounds_checks=True,
            disable_semaphore_checks=True,
        ),
    )(q.reshape(G, _F, D), k.reshape(G, Sk, D), v.reshape(G, Sk, D))
    return out.reshape(B, Hq, Sq, D)
```

```python
import functools
import math

import jax
import jax.numpy as jnp
from jax import lax
import jax.experimental.pallas as pl
import jax.experimental.pallas.tpu as pltpu

_F = 1024
_GS = 8
_R = 8
_DEFER = 2
_LAST_CHUNK = 64


def _qa(j): return ("qka", j, 0, _F)
def _qb(j): return ("qkb", j, 0, _F)
def _pa(j): return ("pva", j, 0, _F)
def _pb(j): return ("pvb", j, 0, _F)
def _sm(j, r=0, t=_F): return ("sm", j, r, t)
def _qk(j, r, t): return ("qk", j, r, t)
def _pv(j, r, t): return ("pv", j, r, t)


def _interleaved(js):
    ops = []
    for n, j in enumerate(js):
        ops.append(_qa(j))
        if n:
            ops.append(_pa(js[n - 1]))
        ops += [_qb(j), _sm(j)]
        if n:
            ops.append(_pb(js[n - 1]))
    return ops + [_pa(js[-1]), _pb(js[-1])]


_RAMP = (
    ([("k", 0, 1), ("qr", 0, 0, 384)],
     [_qk(0, 0, 192), _sm(0, 0, 192), _qk(0, 192, 192)]),
    ([("qr", 0, 384, 384), ("v", 0, 1)],
     [_pv(0, 0, 192), _sm(0, 192, 192), _qk(0, 384, 384), _sm(0, 384, 384),
      _pv(0, 192, 192), _pv(0, 384, 384)]),
    ([("qr", 0, 768, 256), ("k", 1, 1), ("q", 1, 1), ("v", 1, 1)],
     [_qa(1), _qb(1), _sm(1), _qk(0, 768, 256), _sm(0, 768, 256), _pa(1),
      _pv(0, 768, 256)]),
    ([("k", 2, 2), ("q", 2, 2), ("v", 2, 2)],
     [_pb(1)] + _interleaved([2, 3])[:-1]),
    ([("k", 4, 4), ("q", 4, 4), ("v", 4, 4), ("kh", _R, 0, _R)],
     [_pb(3)] + _interleaved([4, 5, 6, 7])),
)


def _attn_kernel(q_hbm, k_hbm, v_hbm, o_hbm, buf, kt, isem, osem, *, c, sk, groups):
    d = buf.shape[2]
    k0, v0 = _F, _F + sk
    hk = sk // 2
    nsteady = (groups - _R) // _GS
    nr = len(_RAMP)
    nt = (((1,), (1,)), ((), ()))

    def piece_copy(p, sem):
        if p[0] == "qr":
            rows = pl.ds(p[2], p[3])
            return pltpu.make_async_copy(q_hbm.at[p[1], rows], buf.at[p[1], rows], sem)
        if p[0] == "kh":
            return pltpu.make_async_copy(k_hbm.at[p[3], pl.ds(p[2] * hk, hk)],
                                         buf.at[p[1], pl.ds(k0 + p[2] * hk, hk)], sem)
        src, off, n = {"q": (q_hbm, 0, _F), "k": (k_hbm, k0, sk), "v": (v_hbm, v0, sk)}[p[0]]
        grp = pl.ds(p[1], p[2])
        return pltpu.make_async_copy(src.at[grp], buf.at[grp, pl.ds(off, n)], sem)

    def steady_pieces(a, nxt):
        return [("kh", a, 1, a), ("k", a + 1, _GS - 1), ("q", a, _GS), ("v", a, _GS),
                ("kh", a + _GS, 0, nxt)]

    def scores(j, r0, t, lo, hi):
        return lax.dot_general(buf[j, r0:r0 + t, :], buf[j, k0 + lo:k0 + hi, :], nt,
                               preferred_element_type=jnp.float32)

    def softmax(s):
        m = jnp.max(s, axis=-1, keepdims=True)
        p = jnp.exp2((s - m) * c)
        l = jnp.sum(p, axis=-1, keepdims=True)
        r = pl.reciprocal(l, approx=True)
        r = r * (2.0 - l * r)
        return (p * r).astype(jnp.bfloat16)

    def values(p, j, lo, hi):
        return jnp.dot(p, buf[j, v0:v0 + sk, lo:hi], preferred_element_type=jnp.float32)

    def store(o, j, r0, t, chunk):
        o = o.astype(buf.dtype)
        if not chunk:
            buf[j, r0:r0 + t, :] = o
            return
        for u in range(0, t, chunk):
            buf[j, r0 + u:r0 + u + chunk, :] = o[u:u + chunk]
            rows = pl.ds(r0 + u, chunk)
            pltpu.make_async_copy(buf.at[j, rows], o_hbm.at[j, rows], osem.at[0]).start()

    def run_ops(ops, vals, base, send, last=None):
        for op in ops:
            name, j, r0, t = op
            g, key = base + j, (j, r0)
            chunk = (_LAST_CHUNK if op == last else t) if send else 0
            if name == "qk":
                vals[key] = scores(g, r0, t, 0, sk)
            elif name == "qkt":
                vals[key] = jnp.dot(buf[g, r0:r0 + t, :], kt[...],
                                    preferred_element_type=jnp.float32)
            elif name == "qka":
                vals[key] = scores(g, r0, t, 0, hk)
            elif name == "qkb":
                vals[key] = jnp.concatenate([vals[key], scores(g, r0, t, hk, sk)], axis=1)
            elif name == "sm":
                vals[key] = softmax(vals[key])
            elif name == "pv":
                store(values(vals.pop(key), g, 0, d), g, r0, t, chunk)
            elif name == "pva":
                vals[key + ("o",)] = values(vals[key], g, 0, d // 2)
            else:
                o = jnp.concatenate(
                    [vals.pop(key + ("o",)), values(vals.pop(key), g, d // 2, d)], axis=1)
                store(o, g, r0, t, chunk)

    for b in range(nr):
        for p in _RAMP[b][0]:
            piece_copy(p, isem.at[b]).start()
    for s in range(nsteady):
        a = _R + s * _GS
        for p in steady_pieces(a, (a + _GS) % groups):
            piece_copy(p, isem.at[nr + s]).start()

    vals = {}
    for b in range(nr):
        for p in _RAMP[b][0]:
            piece_copy(p, isem.at[b]).wait()
        run_ops(_RAMP[b][1], vals, 0, False)
    assert not vals
    kt[...] = buf[_R, k0:k0 + hk, :].T

    ops = _interleaved(list(range(_GS)))
    ops[0] = ("qkt",) + ops[0][1:]

    def body(s, carry):
        a = _R + s * _GS
        for p in steady_pieces(a, 0):
            piece_copy(p, isem.at[nr + s]).wait()
        sv = {}
        run_ops(ops[:1], sv, a, True)

        @pl.when(s < _R // _DEFER)
        def _():
            grp = pl.ds(s * _DEFER, _DEFER)
            pltpu.make_async_copy(buf.at[grp, pl.ds(0, _F)], o_hbm.at[grp], osem.at[0]).start()

        kt[...] = buf[a + _GS, k0:k0 + hk, :].T
        run_ops(ops[1:], sv, a, True, last=ops[-1])
        return carry

    lax.fori_loop(0, nsteady, body, 0)
    pltpu.make_async_copy(buf.at[pl.ds(0, groups), pl.ds(0, _F)], o_hbm, osem.at[0]).wait()


@jax.jit
def pallas_standalone__gqa_softmax__near_ridge_kernel(
    q: jax.Array,
    k: jax.Array,
    v: jax.Array,
):
    B, Hq, Sq, D = q.shape
    _, Hkv, Sk, _ = k.shape
    rep = Hq // Hkv
    G = B * Hkv
    assert rep * Sq == _F and (G - _R) % _GS == 0 and (G - _R) // _GS >= _R // _DEFER
    c = float(D) ** -0.5 * math.log2(math.e)

    out = pl.pallas_call(
        functools.partial(_attn_kernel, c=c, sk=Sk, groups=G),
        in_specs=[pl.BlockSpec(memory_space=pl.ANY)] * 3,
        out_specs=pl.BlockSpec(memory_space=pl.ANY),
        out_shape=jax.ShapeDtypeStruct((G, _F, D), q.dtype),
        scratch_shapes=[
            pltpu.VMEM((G + 1, _F + 2 * Sk, D), q.dtype),
            pltpu.VMEM((D, Sk // 2), q.dtype),
            pltpu.SemaphoreType.DMA((len(_RAMP) + (G - _R) // _GS,)),
            pltpu.SemaphoreType.DMA((1,)),
        ],
        compiler_params=pltpu.CompilerParams(
            vmem_limit_bytes=120 * 1024 * 1024,
            disable_bounds_checks=True,
            disable_semaphore_checks=True,
        ),
    )(q.reshape(G, _F, D), k.reshape(G, Sk, D), v.reshape(G, Sk, D))
    return out.reshape(B, Hq, Sq, D)
```

```python
import functools
import math

import jax
import jax.numpy as jnp
from jax import lax
import jax.experimental.pallas as pl
import jax.experimental.pallas.tpu as pltpu

_F = 1024
_GS = 8
_R = 8
_DEFER = 2
_LAST_CHUNK = 64


def _qa(j): return ("qka", j, 0, _F)
def _qb(j): return ("qkb", j, 0, _F)
def _pa(j): return ("pva", j, 0, _F)
def _pb(j): return ("pvb", j, 0, _F)
def _sm(j, r=0, t=_F): return ("sm", j, r, t)
def _qk(j, r, t): return ("qk", j, r, t)
def _pv(j, r, t): return ("pv", j, r, t)


def _interleaved(js):
    ops = []
    for n, j in enumerate(js):
        ops.append(_qa(j))
        if n:
            ops.append(_pa(js[n - 1]))
        ops += [_qb(j), _sm(j)]
        if n:
            ops.append(_pb(js[n - 1]))
    return ops + [_pa(js[-1]), _pb(js[-1])]


_RAMP = (
    ([("k", 0, 1), ("qr", 0, 0, 384)],
     [_qk(0, 0, 192), _sm(0, 0, 192), _qk(0, 192, 192)]),
    ([("qr", 0, 384, 384), ("v", 0, 1)],
     [_pv(0, 0, 192), _sm(0, 192, 192), _qk(0, 384, 384), _sm(0, 384, 384),
      _pv(0, 192, 192), _pv(0, 384, 384)]),
    ([("qr", 0, 768, 256), ("k", 1, 1), ("q", 1, 1), ("v", 1, 1)],
     [_qa(1), _qb(1), _sm(1), _qk(0, 768, 256), _sm(0, 768, 256), _pa(1),
      _pv(0, 768, 256)]),
    ([("k", 2, 2), ("q", 2, 2), ("v", 2, 2)],
     [_pb(1)] + _interleaved([2, 3])[:-1]),
    ([("k", 4, 4), ("q", 4, 4), ("v", 4, 4), ("kh", _R, 0, _R)],
     [_pb(3)] + _interleaved([4, 5, 6, 7])),
)


def _attn_kernel(q_hbm, k_hbm, v_hbm, o_hbm, buf, kt, isem, osem, *, c, sk, groups):
    d = buf.shape[2]
    k0, v0 = _F, _F + sk
    hk = sk // 2
    nsteady = (groups - _R) // _GS
    nr = len(_RAMP)
    nt = (((1,), (1,)), ((), ()))

    def piece_copy(p, sem):
        if p[0] == "qr":
            rows = pl.ds(p[2], p[3])
            return pltpu.make_async_copy(q_hbm.at[p[1], rows], buf.at[p[1], rows], sem)
        if p[0] == "kh":
            return pltpu.make_async_copy(k_hbm.at[p[3], pl.ds(p[2] * hk, hk)],
                                         buf.at[p[1], pl.ds(k0 + p[2] * hk, hk)], sem)
        src, off, n = {"q": (q_hbm, 0, _F), "k": (k_hbm, k0, sk), "v": (v_hbm, v0, sk)}[p[0]]
        grp = pl.ds(p[1], p[2])
        return pltpu.make_async_copy(src.at[grp], buf.at[grp, pl.ds(off, n)], sem)

    def steady_pieces(a):
        return [("kh", a, 1, a), ("k", a + 1, _GS - 1), ("q", a, _GS), ("v", a, _GS),
                ("kh", a + _GS, 0, (a + _GS) % groups)]

    def scores(j, r0, t, lo, hi):
        return lax.dot_general(buf[j, r0:r0 + t, :], buf[j, k0 + lo:k0 + hi, :], nt,
                               preferred_element_type=jnp.float32)

    def softmax(s):
        m = jnp.max(s, axis=-1, keepdims=True)
        p = jnp.exp2((s - m) * c)
        l = jnp.sum(p, axis=-1, keepdims=True)
        r = pl.reciprocal(l, approx=True)
        r = r * (2.0 - l * r)
        return (p * r).astype(jnp.bfloat16)

    def values(p, j, lo, hi):
        return jnp.dot(p, buf[j, v0:v0 + sk, lo:hi], preferred_element_type=jnp.float32)

    def store(o, j, r0, t, chunk):
        o = o.astype(buf.dtype)
        if not chunk:
            buf[j, r0:r0 + t, :] = o
            return
        for u in range(0, t, chunk):
            buf[j, r0 + u:r0 + u + chunk, :] = o[u:u + chunk]
            rows = pl.ds(r0 + u, chunk)
            pltpu.make_async_copy(buf.at[j, rows], o_hbm.at[j, rows], osem.at[0]).start()

    def run_ops(ops, vals, base, send, last=None):
        for op in ops:
            name, j, r0, t = op
            g, key = base + j, (j, r0)
            chunk = (_LAST_CHUNK if op == last else t) if send else 0
            if name == "qk":
                vals[key] = scores(g, r0, t, 0, sk)
            elif name == "qkt":
                vals[key] = jnp.dot(buf[g, r0:r0 + t, :], kt[...],
                                    preferred_element_type=jnp.float32)
            elif name == "qka":
                vals[key] = scores(g, r0, t, 0, hk)
            elif name == "qkb":
                vals[key] = jnp.concatenate([vals[key], scores(g, r0, t, hk, sk)], axis=1)
            elif name == "sm":
                vals[key] = softmax(vals[key])
            elif name == "pv":
                store(values(vals.pop(key), g, 0, d), g, r0, t, chunk)
            elif name == "pva":
                vals[key + ("o",)] = values(vals[key], g, 0, d // 2)
            else:
                o = jnp.concatenate(
                    [vals.pop(key + ("o",)), values(vals.pop(key), g, d // 2, d)], axis=1)
                store(o, g, r0, t, chunk)

    for b in range(nr):
        for p in _RAMP[b][0]:
            piece_copy(p, isem.at[b]).start()
    for s in range(nsteady):
        for p in steady_pieces(_R + s * _GS):
            piece_copy(p, isem.at[nr + s]).start()

    vals = {}
    for b in range(nr):
        for p in _RAMP[b][0]:
            piece_copy(p, isem.at[b]).wait()
        run_ops(_RAMP[b][1], vals, 0, False)
    assert not vals
    kt[...] = buf[_R, k0:k0 + hk, :].T

    ops = _interleaved(list(range(_GS)))
    ops[0] = ("qkt",) + ops[0][1:]

    def body(s, carry):
        a = _R + s * _GS
        for p in steady_pieces(a):
            piece_copy(p, isem.at[nr + s]).wait()
        sv = {}
        run_ops(ops[:1], sv, a, True)

        @pl.when(s < _R // _DEFER)
        def _():
            grp = pl.ds(s * _DEFER, _DEFER)
            pltpu.make_async_copy(buf.at[grp, pl.ds(0, _F)], o_hbm.at[grp], osem.at[0]).start()

        kt[...] = buf[a + _GS, k0:k0 + hk, :].T
        run_ops(ops[1:], sv, a, True, last=ops[-1])
        return carry

    lax.fori_loop(0, nsteady, body, 0)
    pltpu.make_async_copy(buf.at[pl.ds(0, groups), pl.ds(0, _F)], o_hbm, osem.at[0]).wait()


@jax.jit
def pallas_standalone__gqa_softmax__near_ridge_kernel(
    q: jax.Array,
    k: jax.Array,
    v: jax.Array,
):
    B, Hq, Sq, D = q.shape
    _, Hkv, Sk, _ = k.shape
    rep = Hq // Hkv
    G = B * Hkv
    assert rep * Sq == _F and (G - _R) % _GS == 0 and (G - _R) // _GS >= _R // _DEFER
    c = float(D) ** -0.5 * math.log2(math.e)

    out = pl.pallas_call(
        functools.partial(_attn_kernel, c=c, sk=Sk, groups=G),
        in_specs=[pl.BlockSpec(memory_space=pl.ANY)] * 3,
        out_specs=pl.BlockSpec(memory_space=pl.ANY),
        out_shape=jax.ShapeDtypeStruct((G, _F, D), q.dtype),
        scratch_shapes=[
            pltpu.VMEM((G + 1, _F + 2 * Sk, D), q.dtype),
            pltpu.VMEM((D, Sk // 2), q.dtype),
            pltpu.SemaphoreType.DMA((len(_RAMP) + (G - _R) // _GS,)),
            pltpu.SemaphoreType.DMA((1,)),
        ],
        compiler_params=pltpu.CompilerParams(
            vmem_limit_bytes=120 * 1024 * 1024,
            disable_bounds_checks=True,
            disable_semaphore_checks=True,
        ),
    )(q.reshape(G, _F, D), k.reshape(G, Sk, D), v.reshape(G, Sk, D))
    return out.reshape(B, Hq, Sq, D)
```
